```python
import os as _os
_os.environ.setdefault("JAX_PLATFORMS", "cpu")
import jax
import jax.numpy as jnp

def _softmax(x, axis=-1):
    return jax.nn.softmax(x, axis=axis)
def _gelu(x):
    return jax.nn.gelu(x, approximate=True)
def _silu(x):
    return jax.nn.silu(x)
def _sigmoid(x):
    return jax.nn.sigmoid(x)
def _layernorm(x, axis=-1, eps=1e-5):
    m = jnp.mean(x, axis=axis, keepdims=True)
    v = jnp.var(x, axis=axis, keepdims=True)
    return (x - m) / jnp.sqrt(v + eps)
def _scatter_add(tgt, idx, src, axis=0):
    return tgt.at[idx].add(src)
def _segment_sum(src, seg, n):
    return jax.ops.segment_sum(src, seg, n)
class _Rng:
    def __init__(self, key):
        self._k = key
    def _next(self):
        self._k, sub = jax.random.split(self._k)
        return sub
    def normal(self, shape):
        return jax.random.normal(self._next(), shape, dtype=jnp.bfloat16)
    def randint(self, lo, hi, shape):
        return jax.random.randint(self._next(), shape, lo, hi, dtype=jnp.int32)
    def uniform(self, shape, lo=0.0, hi=1.0):
        return jax.random.uniform(self._next(), shape, jnp.bfloat16, lo, hi)
    def permutation(self, n):
        return jax.random.permutation(self._next(), n)


kernel_name = 'concat_heads__sliding_block_cached__sliding_block_cached__decode'

def setup_inputs():
    _rng = _Rng(jax.random.key(int.from_bytes(__import__("os").urandom(4), "little")))
    _w = (lambda a: (lambda t: t.astype(jnp.bfloat16) if jnp.issubdtype(t.dtype, jnp.floating) else t)(jnp.asarray(a)))
    def _A_setup():
        B, Sq, D = 2, 1, 640
        Hq, Hkv, Sk, Dh = 32, 32, 4096, 128
        assert Hq % Hkv == 0, (Hq, Hkv)
        return {
            "x": _w((lambda *s: _rng.normal(s) * 0.8)(B, Sq, D)),
            "k_cache": _w((lambda *s: _rng.normal(s) * 0.8)(B, Hkv, Sk, Dh)),
            "v_cache": _w((lambda *s: _rng.normal(s) * 0.05)(B, Hkv, Sk, Dh)),
            "wq": _w((lambda *s: _rng.normal(s) * 0.8)(D, Hq * Dh) * (D ** -0.5)),
            "wo": _w((lambda *s: _rng.normal(s) * 0.05)(Hq * Dh, D) * ((Hq * Dh) ** -0.5)),
        }
    _A_in = _A_setup()

    def _B_setup():
        B, Sq, D = 2, 1, 640
        Hq, Hkv, Sk, Dh = 32, 32, 4096, 128
        assert Hq % Hkv == 0, (Hq, Hkv)
        return {
            "x": _w((lambda *s: _rng.normal(s) * 0.8)(B, Sq, D)),
            "k_cache": _w((lambda *s: _rng.normal(s) * 0.8)(B, Hkv, Sk, Dh)),
            "v_cache": _w((lambda *s: _rng.normal(s) * 0.05)(B, Hkv, Sk, Dh)),
            "wq": _w((lambda *s: _rng.normal(s) * 0.8)(D, Hq * Dh) * (D ** -0.5)),
            "wo": _w((lambda *s: _rng.normal(s) * 0.05)(Hq * Dh, D) * ((Hq * Dh) ** -0.5)),
        }
    _B_in = _B_setup()

    return {
        "A_x": _A_in["x"],
        "A_k_cache": _A_in["k_cache"],
        "A_v_cache": _A_in["v_cache"],
        "A_wq": _A_in["wq"],
        "A_wo": _A_in["wo"],
        "B_x": _B_in["x"],
        "B_k_cache": _B_in["k_cache"],
        "B_v_cache": _B_in["v_cache"],
        "B_wq": _B_in["wq"],
        "B_wo": _B_in["wo"],
    }

def reference(A_x, A_k_cache, A_v_cache, A_wq, A_wo, B_x, B_k_cache, B_v_cache, B_wq, B_wo):
    def _A_ref(x, k_cache, v_cache, wq, wo):
        B, Sq, D = x.shape
        Hq, Dh = 32, 128
        Hkv, Sk = k_cache.shape[1], k_cache.shape[2]
        W = min(4096, max(256, Sk // 4))
        rep = Hq // Hkv
        q = (lambda x, *d: x.transpose(*d))((x @ wq).reshape(B, Sq, Hq, Dh), 0, 2, 1, 3)
        k = jnp.repeat(k_cache[:, :, Sk - W:, :], rep, axis=1)
        v = jnp.repeat(v_cache[:, :, Sk - W:, :], rep, axis=1)
        scores = jnp.einsum("bhqd,bhkd->bhqk", q, k) * (Dh ** -0.5)
        p = _softmax(scores, axis=-1)
        o = jnp.einsum("bhqk,bhkd->bhqd", p, v)
        return (lambda x, *d: x.transpose(*d))(o, 0, 2, 1, 3).reshape(B, Sq, Hq * Dh) @ wo

    def _B_ref(x, k_cache, v_cache, wq, wo):
        B, Sq, D = x.shape
        Hq, Dh = 32, 128
        Hkv, Sk = k_cache.shape[1], k_cache.shape[2]
        W = min(4096, max(256, Sk // 4))
        rep = Hq // Hkv
        q = (lambda x, *d: x.transpose(*d))((x @ wq).reshape(B, Sq, Hq, Dh), 0, 2, 1, 3)
        k = jnp.repeat(k_cache[:, :, Sk - W:, :], rep, axis=1)
        v = jnp.repeat(v_cache[:, :, Sk - W:, :], rep, axis=1)
        scores = jnp.einsum("bhqd,bhkd->bhqk", q, k) * (Dh ** -0.5)
        p = _softmax(scores, axis=-1)
        o = jnp.einsum("bhqk,bhkd->bhqd", p, v)
        return (lambda x, *d: x.transpose(*d))(o, 0, 2, 1, 3).reshape(B, Sq, Hq * Dh) @ wo

    a = _A_ref(A_x, A_k_cache, A_v_cache, A_wq, A_wo)
    b = _B_ref(B_x, B_k_cache, B_v_cache, B_wq, B_wo)
    return jnp.concatenate([a, b], axis=-1)
```

```python
import jax
import jax.numpy as jnp
import jax.experimental.pallas as pl
import jax.experimental.pallas.tpu as pltpu

_L = 2
_SPLIT = 8
_PRIO = (0, 1, 1)
_R = 8


@jax.jit
def pallas_concat_heads__sliding_block_cached__sliding_block_cached__decode_kernel(
    A_x: jax.Array,
    A_k_cache: jax.Array,
    A_v_cache: jax.Array,
    A_wq: jax.Array,
    A_wo: jax.Array,
    B_x: jax.Array,
    B_k_cache: jax.Array,
    B_v_cache: jax.Array,
    B_wq: jax.Array,
    B_wo: jax.Array,
):
    B, Sq, D = A_x.shape
    H, Sk, Dh = A_k_cache.shape[1], A_k_cache.shape[2], A_k_cache.shape[3]
    W = min(4096, max(256, Sk // 4))
    assert B == 2 and Sq == 1 and A_wq.shape == (D, H * Dh) and A_wo.shape == (H * Dh, D)
    L, R, split = _L, _R, _SPLIT
    NS = H
    scale = Dh ** -0.5
    ws = W // split

    def kernel(ax, ak, av, awq, awo, bx, bk, bv, bwq, bwo, o_ref,
               kbuf, vbuf, wqbuf, wobuf, acc_ref, x8_ref, sem):
        ks = (ak, bk); vs = (av, bv); wqs = (awq, bwq); wos = (awo, bwo)
        row_d = jax.lax.broadcasted_iota(jnp.int32, (R, D), 0)
        row_w = jax.lax.broadcasted_iota(jnp.int32, (R, W), 0)
        row_h = jax.lax.broadcasted_iota(jnp.int32, (R, Dh), 0)

        def issue(i, slot):
            cs = []
            for t in range(2):
                cs.append(pltpu.make_async_copy(
                    wqs[t].at[:, pl.ds(i * Dh, Dh)], wqbuf.at[slot, t], sem.at[slot, 0]))
            for t in range(2):
                for b in range(2):
                    for s in range(split):
                        cs.append(pltpu.make_async_copy(
                            ks[t].at[b, i, pl.ds(Sk - W + s * ws, ws), :],
                            kbuf.at[slot, t, b, pl.ds(s * ws, ws), :], sem.at[slot, 0]))
            for t in range(2):
                cs.append(pltpu.make_async_copy(
                    wos[t].at[pl.ds(i * Dh, Dh), :], wobuf.at[slot, t], sem.at[slot, 1]))
            for t in range(2):
                for b in range(2):
                    for s in range(split):
                        cs.append(pltpu.make_async_copy(
                            vs[t].at[b, i, pl.ds(Sk - W + s * ws, ws), :],
                            vbuf.at[slot, t, b, pl.ds(s * ws, ws), :], sem.at[slot, 1]))
            for j, c in enumerate(cs):
                c.start(priority=_PRIO[j % len(_PRIO)])

        def wait_qk(slot):
            pltpu.make_async_copy(wqbuf.at[slot], wqbuf.at[slot], sem.at[slot, 0]).wait()
            pltpu.make_async_copy(kbuf.at[slot], kbuf.at[slot], sem.at[slot, 0]).wait()

        def wait_vo(slot):
            pltpu.make_async_copy(wobuf.at[slot], wobuf.at[slot], sem.at[slot, 1]).wait()
            pltpu.make_async_copy(vbuf.at[slot], vbuf.at[slot], sem.at[slot, 1]).wait()

        for i in range(L):
            issue(i, i)

        acc_ref[...] = jnp.zeros_like(acc_ref)
        for t, xr in enumerate((ax, bx)):
            xf = xr[...].astype(jnp.float32)
            x0 = jnp.broadcast_to(xf[0:1], (R, D))
            x1 = jnp.broadcast_to(xf[1:2], (R, D))
            x8_ref[t] = jnp.where(row_d % 2 == 0, x0, x1).astype(jnp.bfloat16)

        def step(i, carry):
            slot = i % L
            wait_qk(slot)
            S = None
            for t in range(2):
                q = jnp.dot(x8_ref[t], wqbuf[slot, t],
                            preferred_element_type=jnp.float32).astype(jnp.bfloat16)
                for b in range(2):
                    s = jax.lax.dot_general(q, kbuf[slot, t, b], (((1,), (1,)), ((), ())),
                                            preferred_element_type=jnp.float32)
                    S = s if S is None else jnp.where(row_w == 2 * t + b, s, S)
            S = S * scale
            m = jnp.max(S, axis=1, keepdims=True)
            P = jnp.exp(S - m)
            inv = 1.0 / jnp.sum(P, axis=1, keepdims=True)
            Pb = P.astype(jnp.bfloat16)
            wait_vo(slot)
            for t in range(2):
                o0 = jnp.dot(Pb, vbuf[slot, t, 0], preferred_element_type=jnp.float32)
                o1 = jnp.dot(Pb, vbuf[slot, t, 1], preferred_element_type=jnp.float32)
                o = jnp.where(row_h == 2 * t, o0, jnp.where(row_h == 2 * t + 1, o1, 0.0)) * inv
                acc_ref[t] += jnp.dot(o.astype(jnp.bfloat16), wobuf[slot, t],
                                      preferred_element_type=jnp.float32)

            @pl.when(i + L < NS)
            def _():
                issue(i + L, slot)
            return carry

        jax.lax.fori_loop(0, NS, step, 0)

        row2 = jax.lax.broadcasted_iota(jnp.int32, (2, D), 0)
        for t in range(2):
            a = acc_ref[t]
            r0 = jnp.sum(jnp.where(row_d % 2 == 0, a, 0.0), axis=0, keepdims=True)
            r1 = jnp.sum(jnp.where(row_d % 2 == 1, a, 0.0), axis=0, keepdims=True)
            r = jnp.where(row2 == 0, jnp.broadcast_to(r0, (2, D)), jnp.broadcast_to(r1, (2, D)))
            o_ref[:, t * D:(t + 1) * D] = r.astype(o_ref.dtype)

    anyspec = pl.BlockSpec(memory_space=pl.ANY)
    xs = pl.BlockSpec((B, D), lambda: (0, 0))
    out = pl.pallas_call(
        kernel,
        in_specs=[xs, anyspec, anyspec, anyspec, anyspec, xs, anyspec, anyspec, anyspec, anyspec],
        out_specs=pl.BlockSpec((B, 2 * D), lambda: (0, 0)),
        out_shape=jax.ShapeDtypeStruct((B, 2 * D), A_x.dtype),
        scratch_shapes=[pltpu.VMEM((L, 2, 2, W, Dh), jnp.bfloat16),
                        pltpu.VMEM((L, 2, 2, W, Dh), jnp.bfloat16),
                        pltpu.VMEM((L, 2, D, Dh), jnp.bfloat16),
                        pltpu.VMEM((L, 2, Dh, D), jnp.bfloat16),
                        pltpu.VMEM((2, R, D), jnp.float32),
                        pltpu.VMEM((2, R, D), jnp.bfloat16),
                        pltpu.SemaphoreType.DMA((L, 2))],
        compiler_params=pltpu.CompilerParams(vmem_limit_bytes=64 * 1024 * 1024),
    )(A_x.reshape(B, D), A_k_cache, A_v_cache, A_wq, A_wo,
      B_x.reshape(B, D), B_k_cache, B_v_cache, B_wq, B_wo)
    return out.reshape(B, Sq, 2 * D)
```

```python
import functools

import jax
import jax.numpy as jnp
import jax.experimental.pallas as pl
import jax.experimental.pallas.tpu as pltpu

_SPLIT = 8
_PRIO = (1, 0, 0, 1, 1, 1, 1, 0)
_WPRIO = (1, 0)
_R = 8


def _compiler_params():
    kw = dict(vmem_limit_bytes=64 * 1024 * 1024)
    for name in ("disable_bounds_checks", "disable_semaphore_checks"):
        if hasattr(pltpu.CompilerParams, name):
            kw[name] = True
    return pltpu.CompilerParams(**kw)


@jax.jit
def pallas_concat_heads__sliding_block_cached__sliding_block_cached__decode_kernel(
    A_x: jax.Array,
    A_k_cache: jax.Array,
    A_v_cache: jax.Array,
    A_wq: jax.Array,
    A_wo: jax.Array,
    B_x: jax.Array,
    B_k_cache: jax.Array,
    B_v_cache: jax.Array,
    B_wq: jax.Array,
    B_wo: jax.Array,
):
    B, Sq, D = A_x.shape
    H, Sk, Dh = A_k_cache.shape[1], A_k_cache.shape[2], A_k_cache.shape[3]
    W = min(4096, max(256, Sk // 4))
    assert B == 2 and Sq == 1 and H >= 3
    assert A_wq.shape == (D, H * Dh) and A_wo.shape == (H * Dh, D)
    R, split = _R, _SPLIT
    NS = H
    scale = Dh ** -0.5
    ws = W // split

    def kernel(ax, ak, av, awq, awo, bx, bk, bv, bwq, bwo, o_ref,
               kbuf, vbuf, wqbuf, wobuf, acc_ref, x8_ref, xbuf, sem, sem2):
        ks = (ak, bk); vs = (av, bv); wqs = (awq, bwq); wos = (awo, bwo)
        row_d = jax.lax.broadcasted_iota(jnp.int32, (R, D), 0)
        row_w = jax.lax.broadcasted_iota(jnp.int32, (R, W), 0)
        row_h = jax.lax.broadcasted_iota(jnp.int32, (R, Dh), 0)

        def issue_window(src, dst, i, slot, s):
            for t in range(2):
                for b in range(2):
                    for c in range(split):
                        pltpu.make_async_copy(
                            src[t].at[b, i, pl.ds(Sk - W + c * ws, ws), :],
                            dst.at[slot, t, b, pl.ds(c * ws, ws), :], s,
                        ).start(priority=_PRIO[c % len(_PRIO)])

        def issue_k(i, slot):
            issue_window(ks, kbuf, i, slot, sem.at[slot, 0])
            for t in range(2):
                pltpu.make_async_copy(wqs[t].at[:, pl.ds(i * Dh, Dh)], wqbuf.at[slot, t],
                                      sem.at[slot, 0]).start(priority=_WPRIO[t])

        def issue_v(i, slot):
            issue_window(vs, vbuf, i, slot, sem.at[slot, 1])
            for t in range(2):
                pltpu.make_async_copy(wos[t].at[pl.ds(i * Dh, Dh), :], wobuf.at[slot, t],
                                      sem.at[slot, 1]).start(priority=_WPRIO[t])

        def wait_k(slot):
            pltpu.make_async_copy(wqbuf.at[slot], wqbuf.at[slot], sem.at[slot, 0]).wait()
            pltpu.make_async_copy(kbuf.at[slot], kbuf.at[slot], sem.at[slot, 0]).wait()

        def wait_v(slot, with_wo=True):
            if with_wo:
                pltpu.make_async_copy(wobuf.at[slot], wobuf.at[slot], sem.at[slot, 1]).wait()
            pltpu.make_async_copy(vbuf.at[slot], vbuf.at[slot], sem.at[slot, 1]).wait()

        def qk(slot, rows):
            S = None
            for t in range(2):
                q = jnp.dot(x8_ref[t], wqbuf[slot, t],
                            preferred_element_type=jnp.float32).astype(jnp.bfloat16)
                for b in range(2):
                    s = jax.lax.dot_general(q, kbuf[slot, t, b], (((1,), (1,)), ((), ())),
                                            preferred_element_type=jnp.float32)
                    S = s if S is None else jnp.where(row_w == rows[t] + b, s, S)
            S = S * scale
            m = jnp.max(S, axis=1, keepdims=True)
            P = jnp.exp(S - m)
            inv = 1.0 / jnp.sum(P, axis=1, keepdims=True)
            return P.astype(jnp.bfloat16), inv

        def pv(slot, Pb, inv, t, rows):
            o0 = jnp.dot(Pb, vbuf[slot, t, 0], preferred_element_type=jnp.float32)
            o1 = jnp.dot(Pb, vbuf[slot, t, 1], preferred_element_type=jnp.float32)
            o = jnp.where(row_h == rows[t], o0, jnp.where(row_h == rows[t] + 1, o1, 0.0)) * inv
            return o.astype(jnp.bfloat16)

        def oproj(slot, o, t):
            return jnp.dot(o, wobuf[slot, t], preferred_element_type=jnp.float32)

        def fold(a):
            row2 = jax.lax.broadcasted_iota(jnp.int32, (2, D), 0)
            r0 = jnp.sum(jnp.where(row_d % 2 == 0, a, 0.0), axis=0, keepdims=True)
            r1 = jnp.sum(jnp.where(row_d % 2 == 1, a, 0.0), axis=0, keepdims=True)
            return jnp.where(row2 == 0, jnp.broadcast_to(r0, (2, D)), jnp.broadcast_to(r1, (2, D)))

        xcs = [pltpu.make_async_copy(xr, xbuf.at[t], sem2.at[0]) for t, xr in enumerate((ax, bx))]
        for c in xcs:
            c.start()
        issue_k(0, 0)
        issue_v(0, 0)
        issue_k(1, 1)
        for c in xcs:
            c.wait()
        acc_ref[...] = jnp.zeros_like(acc_ref)
        for t in range(2):
            xf = xbuf[t].astype(jnp.float32)
            x0 = jnp.broadcast_to(xf[0:1], (R, D))
            x1 = jnp.broadcast_to(xf[1:2], (R, D))
            x8_ref[t] = jnp.where(row_d % 2 == 0, x0, x1).astype(jnp.bfloat16)

        rows = (0, 2)

        def body(i, carry):
            slot = i % 2
            wait_k(slot)
            issue_v(i + 1, 1 - slot)
            Pb, inv = qk(slot, rows)
            wait_v(slot)
            issue_k(i + 2, slot)
            for t in range(2):
                acc_ref[t] += oproj(slot, pv(slot, Pb, inv, t, rows), t)
            return carry

        jax.lax.fori_loop(0, NS - 2, body, 0)

        slot = (NS - 2) % 2
        wait_k(slot)
        issue_window(vs, vbuf, NS - 1, 1 - slot, sem.at[1 - slot, 1])
        Pb, inv = qk(slot, rows)
        wait_v(slot)
        for t in range(2):
            pltpu.make_async_copy(wos[t].at[pl.ds((NS - 1) * Dh, Dh), :], wobuf.at[1 - slot, t],
                                  sem2.at[1 + t]).start(priority=1)
        for t in range(2):
            acc_ref[t] += oproj(slot, pv(slot, Pb, inv, t, rows), t)

        slot = (NS - 1) % 2
        rows = (2, 0)
        wait_k(slot)
        Pb, inv = qk(slot, rows)
        wait_v(slot, with_wo=False)
        o_last = [pv(slot, Pb, inv, t, rows) for t in range(2)]
        acc_b = fold(acc_ref[1])
        for t in range(2):
            pltpu.make_async_copy(wobuf.at[slot, t], wobuf.at[slot, t], sem2.at[1 + t]).wait()
            r = oproj(slot, o_last[t], t)
            r = fold(acc_ref[0] + r) if t == 0 else acc_b + r[0:2]
            o_ref[:, t * D:(t + 1) * D] = r.astype(o_ref.dtype)

    anyspec = pl.BlockSpec(memory_space=pl.ANY)
    out = pl.pallas_call(
        kernel,
        in_specs=[anyspec] * 10,
        out_specs=pl.BlockSpec((B, 2 * D), lambda: (0, 0)),
        out_shape=jax.ShapeDtypeStruct((B, 2 * D), A_x.dtype),
        scratch_shapes=[pltpu.VMEM((2, 2, 2, W, Dh), jnp.bfloat16),
                        pltpu.VMEM((2, 2, 2, W, Dh), jnp.bfloat16),
                        pltpu.VMEM((2, 2, D, Dh), jnp.bfloat16),
                        pltpu.VMEM((2, 2, Dh, D), jnp.bfloat16),
                        pltpu.VMEM((2, R, D), jnp.float32),
                        pltpu.VMEM((2, R, D), jnp.bfloat16),
                        pltpu.VMEM((2, B, D), jnp.bfloat16),
                        pltpu.SemaphoreType.DMA((2, 2)),
                        pltpu.SemaphoreType.DMA((3,))],
        compiler_params=_compiler_params(),
    )(A_x.reshape(B, D), A_k_cache, A_v_cache, A_wq, A_wo,
      B_x.reshape(B, D), B_k_cache, B_v_cache, B_wq, B_wo)
    return out.reshape(B, Sq, 2 * D)
```

```python
import jax
import jax.numpy as jnp
import jax.experimental.pallas as pl
import jax.experimental.pallas.tpu as pltpu

_SPLIT = 16
_UNIT_ORDER = (5, 6, 7, 3, 4, 0, 1, 2)
_QR, _QC = 8, 1024
_OROWS = 16
_R = 8


def _compiler_params():
    kw = dict(vmem_limit_bytes=64 * 1024 * 1024)
    for name in ("disable_bounds_checks", "disable_semaphore_checks"):
        if hasattr(pltpu.CompilerParams, name):
            kw[name] = True
    return pltpu.CompilerParams(**kw)


@jax.jit
def pallas_concat_heads__sliding_block_cached__sliding_block_cached__decode_kernel(
    A_x: jax.Array,
    A_k_cache: jax.Array,
    A_v_cache: jax.Array,
    A_wq: jax.Array,
    A_wo: jax.Array,
    B_x: jax.Array,
    B_k_cache: jax.Array,
    B_v_cache: jax.Array,
    B_wq: jax.Array,
    B_wo: jax.Array,
):
    B, Sq, D = A_x.shape
    H, Sk, Dh = A_k_cache.shape[1], A_k_cache.shape[2], A_k_cache.shape[3]
    W = min(4096, max(256, Sk // 4))
    assert B == 2 and Sq == 1 and H >= 3 and H % 4 == 0
    assert A_wq.shape == (D, H * Dh) and A_wo.shape == (H * Dh, D)
    R, split = _R, _SPLIT
    NS = H
    scale = Dh ** -0.5
    ws = W // split
    per = split // len(_UNIT_ORDER)
    order = tuple(u * per + j for u in _UNIT_ORDER for j in range(per))
    prio = (1, 0)

    def kernel(ax, ak, av, awq, awo, bx, bk, bv, bwq, bwo, o_ref,
               kbuf, vbuf, wqall, wobuf, qbuf, acc_ref, xbuf, sem, sem2):
        ks = (ak, bk); vs = (av, bv); wqs = (awq, bwq); wos = (awo, bwo)
        row_d = jax.lax.broadcasted_iota(jnp.int32, (R, D), 0)
        row_w = jax.lax.broadcasted_iota(jnp.int32, (R, W), 0)
        row_h = jax.lax.broadcasted_iota(jnp.int32, (R, Dh), 0)
        rows = (0, 2)

        def issue_win(src, dst, i, slot, s):
            for b in range(2):
                for c in order:
                    for t in range(2):
                        pltpu.make_async_copy(
                            src[t].at[b, i, pl.ds(Sk - W + c * ws, ws), :],
                            dst.at[slot, t, b, pl.ds(c * ws, ws), :], s,
                        ).start(priority=prio[t])

        def issue_wo(i, slot, sems):
            for r in range(0, Dh, _OROWS):
                for t in range(2):
                    pltpu.make_async_copy(
                        wos[t].at[pl.ds(i * Dh + r, _OROWS), :],
                        wobuf.at[slot, t, pl.ds(r, _OROWS)], sems[t],
                    ).start(priority=prio[t])

        def issue_k(i, slot):
            issue_win(ks, kbuf, i, slot, sem.at[slot, 0])

        def issue_v(i, slot):
            issue_win(vs, vbuf, i, slot, sem.at[slot, 1])
            issue_wo(i, slot, (sem.at[slot, 1], sem.at[slot, 1]))

        def wait_k(slot):
            pltpu.make_async_copy(kbuf.at[slot], kbuf.at[slot], sem.at[slot, 0]).wait()

        def wait_v(slot, with_wo=True):
            if with_wo:
                pltpu.make_async_copy(wobuf.at[slot], wobuf.at[slot], sem.at[slot, 1]).wait()
            pltpu.make_async_copy(vbuf.at[slot], vbuf.at[slot], sem.at[slot, 1]).wait()

        def qproj(t):
            xf = xbuf[t].astype(jnp.float32)
            x0 = jnp.broadcast_to(xf[0:1], (R, D))
            x1 = jnp.broadcast_to(xf[1:2], (R, D))
            x8 = jnp.where(row_d % 2 == 0, x0, x1).astype(jnp.bfloat16)
            for h0 in range(0, H, 4):
                q = jnp.dot(x8, wqall[t, :, h0 * Dh:(h0 + 4) * Dh],
                            preferred_element_type=jnp.float32).astype(jnp.bfloat16)
                for h in range(4):
                    qbuf[t, h0 + h] = q[:, h * Dh:(h + 1) * Dh]

        def qk(i, slot):
            S = None
            for t in range(2):
                q = qbuf[t, i]
                for b in range(2):
                    s = jax.lax.dot_general(q, kbuf[slot, t, b], (((1,), (1,)), ((), ())),
                                            preferred_element_type=jnp.float32)
                    S = s if S is None else jnp.where(row_w == rows[t] + b, s, S)
            S = S * scale
            m = jnp.max(S, axis=1, keepdims=True)
            P = jnp.exp(S - m)
            inv = 1.0 / jnp.sum(P, axis=1, keepdims=True)
            return P.astype(jnp.bfloat16), inv

        def pv(slot, Pb, inv, t):
            o0 = jnp.dot(Pb, vbuf[slot, t, 0], preferred_element_type=jnp.float32)
            o1 = jnp.dot(Pb, vbuf[slot, t, 1], preferred_element_type=jnp.float32)
            o = jnp.where(row_h == rows[t], o0, jnp.where(row_h == rows[t] + 1, o1, 0.0)) * inv
            return o.astype(jnp.bfloat16)

        def oproj(slot, o, t):
            return jnp.dot(o, wobuf[slot, t], preferred_element_type=jnp.float32)

        def pvo(slot, Pb, inv):
            for t in range(2):
                acc_ref[t] += oproj(slot, pv(slot, Pb, inv, t), t)

        def fold(a):
            row2 = jax.lax.broadcasted_iota(jnp.int32, (2, D), 0)
            r0 = jnp.sum(jnp.where(row_d % 2 == 0, a, 0.0), axis=0, keepdims=True)
            r1 = jnp.sum(jnp.where(row_d % 2 == 1, a, 0.0), axis=0, keepdims=True)
            return jnp.where(row2 == 0, jnp.broadcast_to(r0, (2, D)), jnp.broadcast_to(r1, (2, D)))

        xcs = [pltpu.make_async_copy(xr, xbuf.at[t], sem2.at[0]) for t, xr in enumerate((ax, bx))]
        for c in xcs:
            c.start()

        def wq_rows(j, carry):
            r = pl.multiple_of(j * _QR, _QR)
            for cc in range(0, H * Dh, _QC):
                for t in range(2):
                    pltpu.make_async_copy(
                        wqs[t].at[pl.ds(r, _QR), pl.ds(cc, _QC)],
                        wqall.at[t, pl.ds(r, _QR), pl.ds(cc, _QC)], sem2.at[1 + t],
                    ).start(priority=prio[t])
            return carry

        jax.lax.fori_loop(0, D // _QR, wq_rows, 0)
        issue_k(0, 0)
        for c in xcs:
            c.wait()
        acc_ref[...] = jnp.zeros_like(acc_ref)
        pltpu.make_async_copy(wqall.at[1], wqall.at[1], sem2.at[2]).wait()
        issue_v(0, 0)
        qproj(1)
        pltpu.make_async_copy(wqall.at[0], wqall.at[0], sem2.at[1]).wait()
        issue_k(1, 1)
        qproj(0)

        def body(i, carry):
            slot = i % 2
            wait_k(slot)
            issue_v(i + 1, 1 - slot)
            Pb, inv = qk(i, slot)
            wait_v(slot)
            issue_k(i + 2, slot)
            pvo(slot, Pb, inv)
            return carry

        jax.lax.fori_loop(0, NS - 2, body, 0)

        slot = (NS - 2) % 2
        wait_k(slot)
        issue_win(vs, vbuf, NS - 1, 1 - slot, sem.at[1 - slot, 1])
        Pb, inv = qk(NS - 2, slot)
        wait_v(slot)
        issue_wo(NS - 1, 1 - slot, (sem2.at[1], sem2.at[2]))
        pvo(slot, Pb, inv)

        slot = (NS - 1) % 2
        wait_k(slot)
        Pb, inv = qk(NS - 1, slot)
        wait_v(slot, with_wo=False)
        o_last = [pv(slot, Pb, inv, t) for t in range(2)]
        acc_a = fold(acc_ref[0])
        for t in (1, 0):
            pltpu.make_async_copy(wobuf.at[slot, t], wobuf.at[slot, t], sem2.at[1 + t]).wait()
            r = oproj(slot, o_last[t], t)
            r = fold(acc_ref[1] + r) if t == 1 else acc_a + r[0:2]
            o_ref[:, t * D:(t + 1) * D] = r.astype(o_ref.dtype)

    anyspec = pl.BlockSpec(memory_space=pl.ANY)
    out = pl.pallas_call(
        kernel,
        in_specs=[anyspec] * 10,
        out_specs=pl.BlockSpec((B, 2 * D), lambda: (0, 0)),
        out_shape=jax.ShapeDtypeStruct((B, 2 * D), A_x.dtype),
        scratch_shapes=[pltpu.VMEM((2, 2, 2, W, Dh), jnp.bfloat16),
                        pltpu.VMEM((2, 2, 2, W, Dh), jnp.bfloat16),
                        pltpu.VMEM((2, D, H * Dh), jnp.bfloat16),
                        pltpu.VMEM((2, 2, Dh, D), jnp.bfloat16),
                        pltpu.VMEM((2, H, R, Dh), jnp.bfloat16),
                        pltpu.VMEM((2, R, D), jnp.float32),
                        pltpu.VMEM((2, B, D), jnp.bfloat16),
                        pltpu.SemaphoreType.DMA((2, 2)),
                        pltpu.SemaphoreType.DMA((3,))],
        compiler_params=_compiler_params(),
    )(A_x.reshape(B, D), A_k_cache, A_v_cache, A_wq, A_wo,
      B_x.reshape(B, D), B_k_cache, B_v_cache, B_wq, B_wo)
    return out.reshape(B, Sq, 2 * D)
```
